```python
import os as _os
_os.environ.setdefault("JAX_PLATFORMS", "cpu")
import jax
import jax.numpy as jnp

def _softmax(x, axis=-1):
    return jax.nn.softmax(x, axis=axis)
def _gelu(x):
    return jax.nn.gelu(x, approximate=True)
def _silu(x):
    return jax.nn.silu(x)
def _sigmoid(x):
    return jax.nn.sigmoid(x)
def _layernorm(x, axis=-1, eps=1e-5):
    m = jnp.mean(x, axis=axis, keepdims=True)
    v = jnp.var(x, axis=axis, keepdims=True)
    return (x - m) / jnp.sqrt(v + eps)
def _scatter_add(tgt, idx, src, axis=0):
    return tgt.at[idx].add(src)
def _segment_sum(src, seg, n):
    return jax.ops.segment_sum(src, seg, n)
class _Rng:
    def __init__(self, key):
        self._k = key
    def _next(self):
        self._k, sub = jax.random.split(self._k)
        return sub
    def normal(self, shape):
        return jax.random.normal(self._next(), shape, dtype=jnp.bfloat16)
    def randint(self, lo, hi, shape):
        return jax.random.randint(self._next(), shape, lo, hi, dtype=jnp.int32)
    def uniform(self, shape, lo=0.0, hi=1.0):
        return jax.random.uniform(self._next(), shape, jnp.bfloat16, lo, hi)
    def permutation(self, n):
        return jax.random.permutation(self._next(), n)


kernel_name = 'gated_mix__mha_block__ssm_conv_h3__prompt'

def setup_inputs():
    _rng = _Rng(jax.random.key(int.from_bytes(__import__("os").urandom(4), "little")))
    _w = (lambda a: (lambda t: t.astype(jnp.bfloat16) if jnp.issubdtype(t.dtype, jnp.floating) else t)(jnp.asarray(a)))
    def _A_setup():
        B, S, D, H = 1, 2048, 640, 32
        return {
            "x": _w((lambda *s: _rng.normal(s) * 0.05)(B, S, D)),
            "wqkv": _w((lambda *s: _rng.normal(s) * 0.4)(D, 3 * D)),
            "wo": _w((lambda *s: _rng.normal(s) * 0.05)(D, D)),
        }
    _A_in = _A_setup()

    def _B_setup():
        B, S, D = 1, 2048, 640
        ks = 4
        return {
            "q": _w((lambda *s: _rng.normal(s) * 0.05)(B, S, D)),
            "k": _w((lambda *s: _rng.normal(s) * 0.4)(B, S, D)),
            "v": _w((lambda *s: _rng.normal(s) * 0.4)(B, S, D)),
            "shift_k": _w((lambda *s: _rng.normal(s) * 0.4)(D, ks) * 0.5),
            "ssm_k": _w((lambda *s: _rng.normal(s) * 0.4)(D, S) * (1.0 / S ** 0.5)),
            "ssm_D": _w((lambda *s: _rng.normal(s) * 0.4)(D)),
        }
    _B_in = _B_setup()

    return {
        "A_x": _A_in["x"],
        "A_wqkv": _A_in["wqkv"],
        "A_wo": _A_in["wo"],
        "B_q": _B_in["q"],
        "B_k": _B_in["k"],
        "B_v": _B_in["v"],
        "B_shift_k": _B_in["shift_k"],
        "B_ssm_k": _B_in["ssm_k"],
        "B_ssm_D": _B_in["ssm_D"],
        "gate_w": _w((lambda *s: _rng.normal(s) * 0.05)(640) * 16.0),
    }

def reference(A_x, A_wqkv, A_wo, B_q, B_k, B_v, B_shift_k, B_ssm_k, B_ssm_D, gate_w):
    def _A_ref(x, wqkv, wo):
        B, S, D = x.shape
        H = 32
        Dh = D // H
        qkv = (lambda x, *d: x.transpose(*d))((x @ wqkv).reshape(B, S, 3, H, Dh), 2, 0, 3, 1, 4)
        q, k, v = qkv[0], qkv[1], qkv[2]
        scores = jnp.einsum("bhqd,bhkd->bhqk", q, k) * (Dh ** -0.5)
        p = _softmax(scores, axis=-1)
        o = jnp.einsum("bhqk,bhkd->bhqd", p, v)
        return (lambda x, *d: x.transpose(*d))(o, 0, 2, 1, 3).reshape(B, S, D) @ wo

    def _B_ref(q, k, v, shift_k, ssm_k, ssm_D):
        B, S, D = q.shape
        ks = shift_k.shape[-1]
        k_pad = jnp.pad(k, ((0, 0), (ks - 1, 0), (0, 0)))
        k_shift = jnp.zeros_like(k)
        for t in range(ks):
            k_shift = k_shift + k_pad[:, t:t + S, :] * shift_k[:, ks - 1 - t][None, None, :]
        kv = k_shift * v
        L = 2 * S
        kv_pad = jnp.pad(kv, ((0, 0), (0, S), (0, 0)))
        kf_pad = jnp.pad(ssm_k, ((0, 0), (0, S)))
        kv_f = (lambda x, axes=(-2,-1): jnp.fft.rfft2(x.astype(jnp.float32), axes=axes))(kv_pad[:, None, :, :], axes=(1, 2))
        kf_f = (lambda x, axes=(-2,-1): jnp.fft.rfft2(x.astype(jnp.float32), axes=axes))(kf_pad[:, None, :], axes=(1, 2))
        kf_f = (lambda x, *d: x.transpose(*d))(kf_f, 1, 2, 0)
        y_f = kv_f * kf_f[None, :, :, :]
        y = (lambda x, s, axes=(-2,-1): jnp.fft.irfft2(x, s=s, axes=axes).astype(jnp.bfloat16))(y_f, (1, L), axes=(1, 2))[:, 0, :S, :]
        y = y + kv * ssm_D[None, None, :]
        return q * y

    x = A_x
    g = _sigmoid((x * gate_w).sum(-1, keepdims=True))
    a = _A_ref(x, A_wqkv, A_wo)
    b = _B_ref(x, B_k, B_v, B_shift_k, B_ssm_k, B_ssm_D)
    return g * a + (1 - g) * b
```

```python
import functools
import math

import jax
import jax.numpy as jnp
import numpy as np
from jax import lax
import jax.experimental.pallas as pl
import jax.experimental.pallas.tpu as pltpu

F32 = jnp.float32
BF16 = jnp.bfloat16

S = 2048
D = 640
H = 32
DH = 20
NG = 6
CB = 128
NB = S // CB
TQ = 512
CK = 256
NC = S // CK
TP = 512

QSCALE = (DH ** -0.5) * math.log2(math.e)
SAFE_HI = 2.0 ** 100
SAFE_LO = 2.0 ** -80

_NT = (((1,), (1,)), ((), ()))
_TN = (((0,), (0,)), ((), ()))


def _win_start(g):
    return min(120 * g, D - 128)


def _dft_mats():
    f = np.arange(CB, dtype=np.float64)[:, None] + 0.5
    t = np.arange(CB, dtype=np.float64)[None, :]
    th = 2.0 * np.pi * f * t / (2 * CB)
    fwd = np.concatenate([np.cos(th), -np.sin(th)], axis=0)
    inv = np.concatenate([np.cos(th).T, -np.sin(th).T], axis=1) / CB
    return jnp.asarray(fwd, dtype=BF16), jnp.asarray(inv, dtype=BF16)


def _kernel(x_ref, wqkv_ref, wo_ref, bk_ref, bv_ref, shk_ref, ssmk_ref, dvec_ref,
            gw_ref, fwd_ref, inv_ref, o_ref,
            wt_s, wk_s, k_s, qt_s, va_s, ot_s, kpad_s, kv_s, u_s, h_s, y_s, flag_s):
    wt_s[0:D, :] = wqkv_ref[:, 0:D].astype(F32).T.astype(BF16)
    wt_s[D:2 * D, :] = wqkv_ref[:, 2 * D:3 * D].astype(F32).T.astype(BF16)
    for g in range(NG):
        w0 = D + _win_start(g)
        wk_s[:, g * 128:(g + 1) * 128] = wqkv_ref[:, w0:w0 + 128]

    row24 = lax.broadcasted_iota(jnp.int32, (24, TP), 0)

    def proj_body(t, c):
        r0 = pl.multiple_of(t * TP, TP)
        xb = x_ref[pl.ds(r0, TP), :]
        kk = jnp.dot(xb, wk_s[...], preferred_element_type=F32)
        for g in range(NG):
            k_s[g, pl.ds(r0, TP), :] = kk[:, g * 128:(g + 1) * 128].astype(BF16)
        qv = lax.dot_general(wt_s[...], xb, _NT, preferred_element_type=F32)
        qt_s[:, pl.ds(r0, TP)] = qv[0:D] * QSCALE
        for j in range(H // 2):
            b = D + 40 * j
            va_s[2 * j, :, pl.ds(r0, TP)] = jnp.where(row24 < DH, qv[b:b + 24], 1.0)
            va_s[2 * j + 1, :, pl.ds(r0, TP)] = jnp.where(row24 >= 4, qv[b + 16:b + 40], 1.0)
        return c

    lax.fori_loop(0, S // TP, proj_body, 0)

    kpad_s[0:8, :] = jnp.zeros((8, D), F32)
    kpad_s[8:8 + S, :] = bk_ref[...].astype(F32)
    eye = (lax.broadcasted_iota(jnp.int32, (8, 4), 0)
           == lax.broadcasted_iota(jnp.int32, (8, 4), 1)).astype(F32)
    shk = lax.dot_general(eye, shk_ref[...].astype(F32), _NT,
                          preferred_element_type=F32)
    sgn = jnp.where(lax.broadcasted_iota(jnp.int32, (CB, D), 0) % 2 == 0, 1.0, -1.0)
    fwd = fwd_ref[...]

    h_prev = None
    for a in range(NB):
        r0 = a * CB
        ks = kpad_s[8 + r0:8 + r0 + CB, :] * shk[0:1]
        for j in range(1, 4):
            ks = ks + kpad_s[8 + r0 - j:8 + r0 - j + CB, :] * shk[j:j + 1]
        kv = ks * bv_ref[r0:r0 + CB, :].astype(F32)
        kv_s[r0:r0 + CB, :] = kv
        u_s[a] = jnp.dot(fwd, kv.astype(BF16), preferred_element_type=F32)
        hh = lax.dot_general(fwd, ssmk_ref[:, r0:r0 + CB], _NT, preferred_element_type=F32)
        if h_prev is None:
            h_s[a] = hh
        else:
            h_s[a, 0:CB, :] = hh[0:CB] - sgn * h_prev[CB:2 * CB]
            h_s[a, CB:2 * CB, :] = hh[CB:2 * CB] + sgn * h_prev[0:CB]
        h_prev = hh

    def prod_body(ft, c):
        fr = pl.multiple_of(ft * 8, 8)
        fi = pl.multiple_of(CB + ft * 8, 8)
        for a in range(NB):
            yr = None
            yi = None
            for j in range(a + 1):
                ur = u_s[a - j, pl.ds(fr, 8), :]
                ui = u_s[a - j, pl.ds(fi, 8), :]
                hr = h_s[j, pl.ds(fr, 8), :]
                hi = h_s[j, pl.ds(fi, 8), :]
                tr = ur * hr - ui * hi
                ti = ur * hi + ui * hr
                yr = tr if yr is None else yr + tr
                yi = ti if yi is None else yi + ti
            y_s[a, pl.ds(fr, 8), :] = yr
            y_s[a, pl.ds(fi, 8), :] = yi
        return c

    lax.fori_loop(0, CB // 8, prod_body, 0)

    row128 = lax.broadcasted_iota(jnp.int32, (128, TQ), 0)
    row8 = lax.broadcasted_iota(jnp.int32, (8, TQ), 0)
    flag_s[...] = jnp.zeros((8, TQ), F32)

    def head_weights(h, q0):
        g = h // 6
        w0 = pl.multiple_of(jnp.minimum(120 * g, D - 128), 8)
        r0 = DH * h - w0
        qw = qt_s[pl.ds(w0, 128), pl.ds(q0, TQ)]
        w = jnp.where((row128 >= r0) & (row128 < r0 + DH), qw, 0.0).astype(BF16)
        return g, w

    def finish_pair(j, q0, oe, oo):
        oe = oe * (1.0 / oe[DH:DH + 1])
        oo = oo * (1.0 / oo[0:1])
        b = pl.multiple_of(40 * j, 8)
        ot_s[pl.ds(b, 16), pl.ds(q0, TQ)] = oe[0:16]
        ot_s[pl.ds(b + 16, 8), pl.ds(q0, TQ)] = jnp.where(row8 < 4, oe[16:24], oo[0:8])
        ot_s[pl.ds(b + 24, 16), pl.ds(q0, TQ)] = oo[8:24]

    def attn_fast(it, c):
        j = it // (S // TQ)
        q0 = pl.multiple_of((it % (S // TQ)) * TQ, TQ)
        gw = [head_weights(2 * j + e, q0) for e in range(2)]
        items = [(e, cc) for e in range(2) for cc in range(NC)]
        ps = {}
        acc = {}

        def qk(e, cc):
            g, w = gw[e]
            s = jnp.dot(k_s[g, cc * CK:(cc + 1) * CK, :], w, preferred_element_type=F32)
            ps[(e, cc)] = jnp.exp2(s)

        def pv(e, cc):
            o = jnp.dot(va_s[2 * j + e, :, cc * CK:(cc + 1) * CK], ps.pop((e, cc)),
                        preferred_element_type=F32)
            acc[e] = o if cc == 0 else acc[e] + o

        for n in range(len(items) + 1):
            if n < len(items):
                qk(*items[n])
            if n >= 1:
                pv(*items[n - 1])
        oe, oo = acc[0], acc[1]
        bad = flag_s[...]
        for o in (oe, oo):
            for r in range(3):
                bad = jnp.where(jnp.abs(o[8 * r:8 * r + 8]) <= SAFE_HI, bad, 1.0)
        lrow = jnp.where(row8 < 4, oo[0:8], oe[16:24])
        bad = jnp.where(lrow >= SAFE_LO, bad, 1.0)
        flag_s[...] = bad
        finish_pair(j, q0, oe, oo)
        return c

    lax.fori_loop(0, (H // 2) * (S // TQ), attn_fast, 0)

    def attn_safe(it, c):
        j = it // (S // TQ)
        q0 = pl.multiple_of((it % (S // TQ)) * TQ, TQ)
        outs = []
        for e in range(2):
            g, w = head_weights(2 * j + e, q0)
            s = jnp.dot(k_s[g], w, preferred_element_type=F32)
            m = jnp.max(s, axis=0, keepdims=True)
            p = jnp.exp2(s - m)
            outs.append(jnp.dot(va_s[2 * j + e], p, preferred_element_type=F32))
        finish_pair(j, q0, outs[0], outs[1])
        return c

    @pl.when(jnp.max(flag_s[...]) > 0.0)
    def _():
        lax.fori_loop(0, (H // 2) * (S // TQ), attn_safe, 0)

    dvec = dvec_ref[...].astype(F32)
    gw_row = gw_ref[...].astype(F32)
    inv = inv_ref[...]

    def epi_body(t, c):
        r0 = pl.multiple_of(t * TP, TP)
        a = lax.dot_general(ot_s[:, pl.ds(r0, TP)].astype(BF16), wo_ref[...], _TN,
                            preferred_element_type=F32)
        for i in range(TP // CB):
            rr = pl.multiple_of(r0 + i * CB, CB)
            yc = jnp.dot(inv, y_s[t * (TP // CB) + i].astype(BF16), preferred_element_type=F32)
            xb = x_ref[pl.ds(rr, CB), :].astype(F32)
            y = yc + kv_s[pl.ds(rr, CB), :] * dvec
            z = jnp.sum(xb * gw_row, axis=-1, keepdims=True)
            g = 1.0 / (1.0 + jnp.exp(-z))
            b = xb * y
            o_ref[pl.ds(rr, CB), :] = (g * a[i * CB:(i + 1) * CB] + (1.0 - g) * b).astype(BF16)
        return c

    lax.fori_loop(0, S // TP, epi_body, 0)


@jax.jit
def pallas_gated_mix__mha_block__ssm_conv_h3__prompt_kernel(
    A_x: jax.Array,
    A_wqkv: jax.Array,
    A_wo: jax.Array,
    B_q: jax.Array,
    B_k: jax.Array,
    B_v: jax.Array,
    B_shift_k: jax.Array,
    B_ssm_k: jax.Array,
    B_ssm_D: jax.Array,
    gate_w: jax.Array,
):
    del B_q
    fwd, inv = _dft_mats()
    vm = pl.BlockSpec(memory_space=pltpu.VMEM)
    out = pl.pallas_call(
        _kernel,
        out_shape=jax.ShapeDtypeStruct((S, D), BF16),
        in_specs=[vm] * 11,
        out_specs=vm,
        scratch_shapes=[
            pltpu.VMEM((2 * D, D), BF16),
            pltpu.VMEM((D, NG * 128), BF16),
            pltpu.VMEM((NG, S, 128), BF16),
            pltpu.VMEM((D, S), F32),
            pltpu.VMEM((H, 24, S), F32),
            pltpu.VMEM((D, S), F32),
            pltpu.VMEM((S + 8, D), F32),
            pltpu.VMEM((S, D), F32),
            pltpu.VMEM((NB, 2 * CB, D), F32),
            pltpu.VMEM((NB, 2 * CB, D), F32),
            pltpu.VMEM((NB, 2 * CB, D), F32),
            pltpu.VMEM((8, TQ), F32),
        ],
        compiler_params=pltpu.CompilerParams(vmem_limit_bytes=120 * 1024 * 1024),
    )(
        A_x.reshape(S, D), A_wqkv, A_wo, B_k.reshape(S, D), B_v.reshape(S, D),
        B_shift_k, B_ssm_k, B_ssm_D.reshape(1, D), gate_w.reshape(1, D), fwd, inv,
    )
    return out.reshape(1, S, D)
```

```python
import functools
import math

import jax
import jax.numpy as jnp
import numpy as np
from jax import lax
import jax.experimental.pallas as pl
import jax.experimental.pallas.tpu as pltpu

F32 = jnp.float32
BF16 = jnp.bfloat16

S = 2048
D = 640
H = 32
DH = 20
NP = H // 2
CB = 128
NB = S // CB
TQ = 512
NT = S // TQ
CK = 128
NC = S // CK
TP = 512
TV = 256
NL = D // 128
NPIECE = 5
RV = 16
VLAG = 2
NSLOT = 4
DEP_LEAD = 2
DEP_TAIL = 0
NV = S // TV
FR = CB // NV

QSCALE = (DH ** -0.5) * math.log2(math.e)
SAFE_HI = 2.0 ** 100
SAFE_LO = 2.0 ** -80

_NT = (((1,), (1,)), ((), ()))
_TN = (((0,), (0,)), ((), ()))


def _rev8(p):
    parts = []
    for t in range(p.shape[0] // 128):
        for g in reversed(range(16)):
            parts.append(p[t * 128 + g * 8:t * 128 + g * 8 + 8])
    return jnp.concatenate(parts, axis=0)


def _dft_mats():
    f = np.arange(CB, dtype=np.float64)[:, None] + 0.5
    t = np.arange(CB, dtype=np.float64)[None, :]
    th = 2.0 * np.pi * f * t / (2 * CB)
    fwd = np.concatenate([np.cos(th), -np.sin(th)], axis=0)
    inv = np.concatenate([np.cos(th).T, -np.sin(th).T], axis=1) / CB
    return jnp.asarray(fwd, dtype=BF16), jnp.asarray(inv, dtype=BF16)


def _kernel(x_hbm, wqkv_hbm, wo_hbm, bk_hbm, bv_hbm, ssmk_hbm,
            shk_ref, dvec_ref, gw_ref, fwd_ref, inv_ref, o_hbm,
            x_v, w_v, wo_v, bk_v, bv_v, ssmk_v, o_v, sems,
            wt_s, xf_s, k_s, qvt_s, ot_s, kpad_s, kv_s, u_s, h_s, y_s, k1_s, flag_s, zero_s, kb_s, pv_s, qc_s):
    NX = S // TP

    def cp(i, src, dst):
        return pltpu.make_async_copy(src, dst, sems.at[i])

    cp_x = [cp(i, x_hbm.at[pl.ds(i * TP, TP), :], x_v.at[pl.ds(i * TP, TP), :]) for i in range(NX)]
    cp_w = [cp(NX + i, wqkv_hbm.at[:, pl.ds(i * D, D)], w_v.at[i]) for i in range(3)]
    cp_h = cp(NX + 3, ssmk_hbm, ssmk_v)
    cp_k = cp(NX + 4, bk_hbm, bk_v)
    cp_v = cp(NX + 5, bv_hbm, bv_v)
    cp_wo = cp(NX + 6, wo_hbm, wo_v)

    def cp_o(i):
        return cp(NX + 7 + i, o_v.at[pl.ds(i * TP, TP), :], o_hbm.at[pl.ds(i * TP, TP), :])

    cp_w[1].start()
    cp_x[0].start()
    cp_w[1].wait()
    cp_x[0].wait()
    for i in range(1, NX):
        cp_x[i].start()
    cp_h.start()

    for t in range(NX):
        if t > 0:
            cp_x[t].wait()
        if t == 1:
            cp_k.start()
            cp_v.start()
        if t == 3:
            cp_w[0].start()
            cp_w[2].start()
            cp_wo.start()
        r0 = t * TP
        kk = jnp.dot(x_v[r0:r0 + TP, :], w_v[1], preferred_element_type=F32)
        kk = _rev8(kk).astype(BF16)
        xf_s[r0:r0 + TP, :] = x_v[r0:r0 + TP, :].astype(F32)
        for j in range(NP):
            if 40 * j + 48 <= D:
                kj = kk[:, 40 * j:40 * j + 48]
            else:
                kj = jnp.concatenate([kk[:, 40 * j:D], kk[:, 0:8]], axis=1)
            k_s[j, r0:r0 + TP, :] = kj

    def scatter(ref, a, re, im):
        for g in range(NV):
            ref[g, a, 0] = re[g * FR:(g + 1) * FR]
            ref[g, a, 1] = im[g * FR:(g + 1) * FR]

    fwd = fwd_ref[...]
    sgn = jnp.where(lax.broadcasted_iota(jnp.int32, (CB, D), 0) % 2 == 0, 1.0, -1.0)
    cp_h.wait()
    h_prev = None
    for a in range(NB):
        r0 = a * CB
        hh = lax.dot_general(fwd, ssmk_v[:, r0:r0 + CB], _NT, preferred_element_type=F32)
        if h_prev is None:
            scatter(h_s, a, hh[0:CB], hh[CB:2 * CB])
        else:
            scatter(h_s, a, hh[0:CB] - sgn * h_prev[CB:2 * CB],
                    hh[CB:2 * CB] + sgn * h_prev[0:CB])
        h_prev = hh

    cp_k.wait()
    cp_v.wait()
    kpad_s[0:8, :] = jnp.zeros((8, D), F32)
    kpad_s[8:8 + S, :] = bk_v[...].astype(F32)
    shk = shk_ref[...].astype(F32)
    for a in range(NB):
        r0 = a * CB
        ks = kpad_s[8 + r0:8 + r0 + CB, :] * shk[0:1]
        for j in range(1, 4):
            ks = ks + kpad_s[8 + r0 - j:8 + r0 - j + CB, :] * shk[j:j + 1]
        kv = ks * bv_v[r0:r0 + CB, :].astype(F32)
        kv_s[r0:r0 + CB, :] = kv
        uu = jnp.dot(fwd, kv.astype(BF16), preferred_element_type=F32)
        scatter(u_s, a, uu[0:CB], uu[CB:2 * CB])

    cp_w[0].wait()
    cp_w[2].wait()
    wt_s[0:D, :] = w_v[0].astype(F32).T
    wt_s[D:2 * D, :] = w_v[2].astype(F32).T

    def conv16(us, hs, init, dep):
        if dep is not None:
            hs = [jnp.where(dep[0], hs[0], dep[1])] + hs[1:]
        outs = []
        for a in range(NB):
            acc = None if init is None else init(a)
            for j in range(a + 1):
                t = us[a - j] * hs[j]
                acc = t if acc is None else acc + t
            outs.append(acc)
        return outs

    def products(t, p, deps):
        rs = slice((p // NL) * 8, (p // NL) * 8 + 8)
        ls = slice((p % NL) * 128, (p % NL + 1) * 128)
        ur = lambda a: u_s[t, a, 0, rs, ls]
        ui = lambda a: u_s[t, a, 1, rs, ls]
        hr = lambda a: h_s[t, a, 0, rs, ls]
        hi = lambda a: h_s[t, a, 1, rs, ls]
        k1 = conv16([ur(a) + ui(a) for a in range(NB)], [hr(a) for a in range(NB)], None, deps[0])
        for a in range(NB):
            k1_s[p, a] = k1[a]
        yi = conv16([ur(a) for a in range(NB)], [hi(a) - hr(a) for a in range(NB)],
                    lambda a: k1_s[p, a], deps[1])
        for a in range(NB):
            y_s[t, a, 1, rs, ls] = yi[a]
        yr = conv16([ui(a) for a in range(NB)], [-hi(a) - hr(a) for a in range(NB)],
                    lambda a: k1_s[p, a], deps[2])
        for a in range(NB):
            y_s[t, a, 0, rs, ls] = yr[a]

    FT = FR // 8
    zero_s[...] = jnp.zeros((8, 128), F32)

    def qv_body(t, c):
        r0 = pl.multiple_of(t * TV, TV)
        xb = xf_s[pl.ds(r0, TV), :]
        always = zero_s[...] == 0.0
        npos = FT * NL
        rows = 2 * D // NPIECE
        tiles = []
        for i in range(NPIECE):
            qv = lax.dot_general(wt_s[i * rows:(i + 1) * rows, :], xb, _NT,
                                 preferred_element_type=F32)
            lo, hi_ = i * rows, (i + 1) * rows
            if hi_ <= D:
                qvt_s[lo:hi_, pl.ds(r0, TV)] = (qv * QSCALE).astype(BF16).astype(F32)
            elif lo >= D:
                qvt_s[lo:hi_, pl.ds(r0, TV)] = qv
            else:
                qvt_s[lo:D, pl.ds(r0, TV)] = (qv[0:D - lo] * QSCALE).astype(BF16).astype(F32)
                qvt_s[D:hi_, pl.ds(r0, TV)] = qv[D - lo:]
            for l in range(TV // 128):
                for r in range(rows // 8):
                    tiles.append(qv[r * 8:(r + 1) * 8, l * 128:(l + 1) * 128])
        ncv = 3 * npos
        for p in range(npos):
            deps = []
            for k in range(3):
                idx = ((3 * p + k - DEP_LEAD) * len(tiles)) // (ncv + DEP_TAIL)
                deps.append(None if idx < 0 else (always, tiles[idx]))
            products(t, p, deps)
        return c

    lax.fori_loop(0, NV, qv_body, 0)

    row8 = lax.broadcasted_iota(jnp.int32, (8, TQ), 0)
    row8k = lax.broadcasted_iota(jnp.int32, (8, CK), 0)
    row8s = lax.broadcasted_iota(jnp.int32, (8, S), 0)
    flag_s[...] = jnp.zeros((8, TQ), F32)

    def head_weights(b, e, qs):
        zeros8 = jnp.zeros((8, TQ), F32)
        mid = qvt_s[pl.ds(b + 16, 8), qs]
        if e == 0:
            w = jnp.concatenate([qvt_s[pl.ds(b, 16), qs],
                                 jnp.where(row8 < 4, mid, 0.0), zeros8], axis=0)
        else:
            w = jnp.concatenate([zeros8, zeros8, jnp.where(row8 >= 4, mid, 0.0),
                                 qvt_s[pl.ds(b + 24, 16), qs], zeros8], axis=0)
        return w.astype(BF16)

    def v_window(b, e, k0, n, rows):
        mid = qvt_s[pl.ds(D + b + 16, 8), k0:k0 + n]
        if e == 0:
            return jnp.concatenate([qvt_s[pl.ds(D + b, 16), k0:k0 + n],
                                    jnp.where(rows < 4, mid, 1.0)], axis=0)
        return jnp.concatenate([jnp.where(rows >= 4, mid, 1.0),
                                qvt_s[pl.ds(D + b + 24, 16), k0:k0 + n]], axis=0)

    def finish_pair(b, qs, oe, oo):
        oe = oe * (1.0 / oe[DH:DH + 1])
        oo = oo * (1.0 / oo[0:1])
        ot_s[pl.ds(b, 16), qs] = oe[0:16]
        ot_s[pl.ds(b + 16, 8), qs] = jnp.where(row8 < 4, oe[16:24], oo[0:8])
        ot_s[pl.ds(b + 24, 16), qs] = oo[8:24]

    def make_kb(jn, e, cc):
        kf = k_s[jn, cc * CK:cc * CK + RV, :].astype(F32)
        for g in range(RV // 8):
            for d in range(DH):
                col = kf[g * 8:(g + 1) * 8, DH * e + d:DH * e + d + 1]
                kb_s[e, cc, g, d] = jnp.broadcast_to(col, (8, 128))

    for e in range(2):
        for cc in range(NC):
            make_kb(0, e, cc)

    def attn_fast(j, c):
        b = pl.multiple_of(40 * j, 8)
        jn = jnp.minimum(j + 1, NP - 1)
        always = zero_s[...] == 0.0
        qc_s[...] = qvt_s[pl.ds(b, 40), :]
        items = [(t, e, cc) for t in range(NT) for e in range(2) for cc in range(NC)]
        ws = {}
        ps = {}
        acc = {}

        def qk(t, e, cc):
            if cc == 0:
                ws[(t, e)] = head_weights(b, e, slice(t * TQ, (t + 1) * TQ))
            w = ws[(t, e)]
            s = jnp.dot(k_s[j, cc * CK + RV:(cc + 1) * CK, 0:w.shape[0]], w,
                        preferred_element_type=F32)
            ps[(t, e, cc)] = jnp.exp2(s)

        def vpu(n, dep):
            t, e, cc = items[n]
            for g in range(RV // 8):
                for lt in range(TQ // 128):
                    a = None
                    for d in range(DH):
                        kb = kb_s[e, cc, g, d]
                        if d == 0 and dep is not None:
                            r = ((g * 4 + lt) * (CK - RV) // 8) // (RV // 2)
                            kb = jnp.where(always, kb, dep[r * 8:r * 8 + 8, 0:128])
                        q0 = t * TQ + lt * 128
                        m = kb * qc_s[DH * e + d:DH * e + d + 1, q0:q0 + 128]
                        a = m if a is None else a + m
                    pv_s[n % NSLOT, g * 8:(g + 1) * 8, lt * 128:(lt + 1) * 128] = jnp.exp2(a)
            if t == NT - 1:
                make_kb(jn, e, cc)

        def pv(n):
            t, e, cc = items[n]
            p = _rev8(jnp.concatenate([pv_s[n % NSLOT], ps[(t, e, cc)]], axis=0))
            o = jnp.dot(v_window(b, e, cc * CK, CK, row8k), p, preferred_element_type=F32)
            acc[e] = o if cc == 0 else acc[e] + o
            if cc == NC - 1 and e == 1:
                oe, oo = acc[0], acc[1]
                bad = flag_s[...]
                for o in (oe, oo):
                    for r in range(3):
                        bad = jnp.where(jnp.abs(o[8 * r:8 * r + 8]) <= SAFE_HI, bad, 1.0)
                lrow = jnp.where(row8 < 4, oo[0:8], oe[16:24])
                bad = jnp.where(lrow >= SAFE_LO, bad, 1.0)
                flag_s[...] = bad
                finish_pair(b, slice(t * TQ, (t + 1) * TQ), oe, oo)

        for n in range(len(items) + 1):
            if n < len(items):
                qk(*items[n])
                vpu(n, ps[items[n - VLAG]] if n >= VLAG else None)
            if n >= 1:
                pv(n - 1)
        return c

    lax.fori_loop(0, NP, attn_fast, 0)

    def attn_safe(it, c):
        j = it // NT
        b = pl.multiple_of(40 * j, 8)
        qs = pl.ds(pl.multiple_of((it % NT) * TQ, TQ), TQ)
        outs = []
        for e in range(2):
            w = head_weights(b, e, qs)
            s = jnp.dot(k_s[j, :, 0:w.shape[0]], w, preferred_element_type=F32)
            m = jnp.max(s, axis=0, keepdims=True)
            p = _rev8(jnp.exp2(s - m))
            outs.append(jnp.dot(v_window(b, e, 0, S, row8s), p, preferred_element_type=F32))
        finish_pair(b, qs, outs[0], outs[1])
        return c

    @pl.when(jnp.max(flag_s[...]) > 0.0)
    def _():
        lax.fori_loop(0, NP * NT, attn_safe, 0)

    dvec = dvec_ref[...].astype(F32)
    gw_row = gw_ref[...].astype(F32)
    inv = inv_ref[...]
    cp_wo.wait()

    def epi_body(t, c):
        r0 = pl.multiple_of(t * TP, TP)
        a = lax.dot_general(ot_s[:, pl.ds(r0, TP)].astype(BF16), wo_v[...], _TN,
                            preferred_element_type=F32)
        for i in range(TP // CB):
            rr = pl.multiple_of(r0 + i * CB, CB)
            ab = t * (TP // CB) + i
            yf = jnp.concatenate([y_s[g, ab, ri] for ri in range(2) for g in range(NV)], axis=0)
            yc = jnp.dot(inv, yf.astype(BF16), preferred_element_type=F32)
            xb = xf_s[pl.ds(rr, CB), :]
            y = yc + kv_s[pl.ds(rr, CB), :] * dvec
            z = jnp.sum(xb * gw_row, axis=-1, keepdims=True)
            g = 1.0 / (1.0 + jnp.exp(-z))
            b = xb * y
            o_v[pl.ds(rr, CB), :] = (g * a[i * CB:(i + 1) * CB] + (1.0 - g) * b).astype(BF16)
        pltpu.make_async_copy(o_v.at[pl.ds(r0, TP), :], o_hbm.at[pl.ds(r0, TP), :],
                              sems.at[NX + 7 + t]).start()
        return c

    lax.fori_loop(0, NX, epi_body, 0)
    for i in range(NX):
        cp_o(i).wait()


@jax.jit
def pallas_gated_mix__mha_block__ssm_conv_h3__prompt_kernel(
    A_x: jax.Array,
    A_wqkv: jax.Array,
    A_wo: jax.Array,
    B_q: jax.Array,
    B_k: jax.Array,
    B_v: jax.Array,
    B_shift_k: jax.Array,
    B_ssm_k: jax.Array,
    B_ssm_D: jax.Array,
    gate_w: jax.Array,
):
    del B_q
    fwd, inv = _dft_mats()
    vm = pl.BlockSpec(memory_space=pltpu.VMEM)
    hbm = pl.BlockSpec(memory_space=pl.ANY)
    out = pl.pallas_call(
        _kernel,
        out_shape=jax.ShapeDtypeStruct((S, D), BF16),
        in_specs=[hbm] * 6 + [vm] * 5,
        out_specs=hbm,
        scratch_shapes=[
            pltpu.VMEM((S, D), BF16),
            pltpu.VMEM((3, D, D), BF16),
            pltpu.VMEM((D, D), BF16),
            pltpu.VMEM((S, D), BF16),
            pltpu.VMEM((S, D), BF16),
            pltpu.VMEM((D, S), BF16),
            pltpu.VMEM((S, D), BF16),
            pltpu.SemaphoreType.DMA((2 * (S // TP) + 7,)),
            pltpu.VMEM((2 * D, D), F32),
            pltpu.VMEM((S, D), F32),
            pltpu.VMEM((NP, S, 48), BF16),
            pltpu.VMEM((2 * D, S), F32),
            pltpu.VMEM((D, S), F32),
            pltpu.VMEM((S + 8, D), F32),
            pltpu.VMEM((S, D), F32),
            pltpu.VMEM((NV, NB, 2, FR, D), F32),
            pltpu.VMEM((NV, NB, 2, FR, D), F32),
            pltpu.VMEM((NV, NB, 2, FR, D), F32),
            pltpu.VMEM((FR // 8 * NL, NB, 8, 128), F32),
            pltpu.VMEM((8, TQ), F32),
            pltpu.VMEM((8, 128), F32),
            pltpu.VMEM((2, NC, RV // 8, DH, 8, 128), F32),
            pltpu.VMEM((NSLOT, RV, TQ), F32),
            pltpu.VMEM((40, S), F32),
        ],
        compiler_params=pltpu.CompilerParams(vmem_limit_bytes=120 * 1024 * 1024),
    )(
        A_x.reshape(S, D), A_wqkv, A_wo, B_k.reshape(S, D), B_v.reshape(S, D), B_ssm_k,
        B_shift_k.T, B_ssm_D.reshape(1, D), gate_w.reshape(1, D), fwd, inv,
    )
    return out.reshape(1, S, D)
```

```python
import math

import jax
import jax.numpy as jnp
import numpy as np
from jax import lax
import jax.experimental.pallas as pl
import jax.experimental.pallas.tpu as pltpu

F32 = jnp.float32
BF16 = jnp.bfloat16

S = 2048
D = 640
H = 32
DH = 20
NP = H // 2
CB = 128
NB = S // CB
TQ = 512
NT = S // TQ
TS = 128
CK = 128
NC = S // CK
TP = 512
TV = 512
NL = D // 128
K4 = D - 128

XCH = (256, 512, 1280)
KSUB = 256
WK0 = 3
KLAST = 256
FORDER = 'huhuhuuh'
QREP = 2
PAT = (3, 2, 3, 2)
DOTS = (14, 14, 14, 12)
TC = len(PAT)
TK = TC * CK
TAU0 = -3.5
LEAD = 8.0
VGD = 10
DEP_LEAD = 1
EG_LEAD = 4
EG_SPAN = 16
EG_X = 4

QSCALE = (DH ** -0.5) * math.log2(math.e)
SAFE_HI = 2.0 ** 100
SAFE_LO = 2.0 ** -40

_NT = (((1,), (1,)), ((), ()))


def _plan():
    order, src_of, md, mo, vof, due = [], [], [], [], [], []
    nvtot = 0
    tbase = 0.0
    need = [16 - v for v in PAT]
    cum = np.cumsum(need)
    assert sum(DOTS) == cum[-1] and all(np.cumsum(DOTS) >= cum)
    for sc in range(NC // TC):
        arr, loc = [], []
        t = tbase
        starts = []
        for i in range(TC):
            starts.append(t)
            for r in range(DOTS[i]):
                arr.append(t + r)
                loc.append((TC * sc + i, r))
            t += DOTS[i] + 3
        span = t - tbase
        nv = sum(PAT)
        vi = 0
        vgroups, mgroups = [], []
        for i in range(TC):
            lo = 0 if i == 0 else int(cum[i - 1])
            ks = []
            for _ in range(PAT[i]):
                tau = tbase + TAU0 + vi * span / nv
                k = sum(1 for r in range(lo, int(cum[i])) if arr[r] < tau)
                k = min(k, need[i] - 1)
                ks.append(k)
                due.append(max(tau, starts[i] - 2.0))
                vi += 1
            vpos = [k + idx for idx, k in enumerate(ks)]
            srcs = {}
            r = lo
            for pos in range(16):
                g = 15 - pos
                if pos in vpos:
                    srcs[g] = ("v", nvtot + len(vgroups))
                    vgroups.append(16 * i + g)
                else:
                    srcs[g] = ("m",) + loc[r]
                    mgroups.append(16 * i + g)
                    r += 1
            src_of.append(srcs)
            vof.append(nvtot + sum(PAT[:i]))
        off = 16 * TC * sc + nv
        for i in range(TC):
            mo.append(off)
            md.append(DOTS[i])
            off += DOTS[i]
        order.append(vgroups + mgroups)
        nvtot += nv
        tbase = t
    vof.append(nvtot)
    times = []
    t = 0.0
    for c in range(NC):
        times += [(t + r, c, r) for r in range(md[c])]
        t += md[c] + 3

    def gate_at(tt):
        wrap = 0
        if tt < 0:
            tt += t
            wrap = -NC
        best = [x for x in times if x[0] <= tt][-1]
        return (best[1] + wrap, best[2])

    gates = [gate_at(tau - LEAD) for tau in due]
    return order, src_of, md, mo, vof, gates, nvtot


ORDER, SRC_OF, MD, MO, VOF, GATES, NG = _plan()
NGP = -(-NG // 4) * 4


def _to_stored(p, sc):
    return jnp.concatenate([p[g * 8:g * 8 + 8] for g in ORDER[sc]], axis=0)


def _to_natural(p):
    parts = []
    n = 16 * TC
    for sc in range(NC // TC):
        pos = {g: i for i, g in enumerate(ORDER[sc])}
        parts += [p[(n * sc + pos[g]) * 8:(n * sc + pos[g]) * 8 + 8] for g in range(n)]
    return jnp.concatenate(parts, axis=0)


def _dft_mats():
    fidx = np.concatenate([np.arange(0, CB, 2), np.arange(1, CB, 2)])
    w = 2.0 * np.pi * (fidx.astype(np.float64)[:, None] + 0.5) / (2 * CB)
    t = np.arange(CB, dtype=np.float64)[None, :]

    def fwd(th):
        return np.stack([np.cos(th).reshape(CB // 8, 8, CB),
                         -np.sin(th).reshape(CB // 8, 8, CB)], axis=1).reshape(2 * CB, CB)

    tau = np.arange(CB // 2, dtype=np.float64)[None, :] + 0.5
    inv = np.concatenate([np.cos(w * tau).T, np.sin(w * tau).T], axis=0) / CB
    return (jnp.asarray(np.stack([fwd(w * t), fwd(w * (t - (CB - 1) / 2))]), dtype=BF16),
            jnp.asarray(inv, dtype=BF16))


def _kernel(x_hbm, wqkv_hbm, wo_hbm, bk_hbm, bv_hbm, ssmk_hbm,
            shk_hbm, dvec_hbm, gw_hbm, fwd_hbm, inv_hbm, o_hbm,
            x_v, wk_v, wc_v, wo_v, bk_v, bv_v, ssmk_v, o_v, sems,
            wt_s, xp_s, k_s, qvt_s, ow_s, u_s, h_s, y_s, cw_s, flag_s, zero_s,
            kb0_s, kb1_s, qc0_s, qc1_s, kf_s, kfc_s, kr_s,
            fwd_ref, inv_ref, shk_ref, dvec_ref, gw_ref, run_s):
    NX = S // TP
    SEM_E = len(XCH)
    SEM_W = SEM_E + 1
    SEM_C = SEM_E + 2

    def cp(i, src, dst):
        return pltpu.make_async_copy(src, dst, sems.at[i])

    cp_xc = []
    r_ = 0
    for ci, n in enumerate(XCH):
        cp_xc.append([cp(ci, x_hbm.at[pl.ds(r_, n), :], x_v.at[pl.ds(r_, n), :])] if ci else [])
        r_ += n
    w0 = WK0 * 128
    cp_w0 = [cp(SEM_W, wqkv_hbm.at[:, pl.ds(D, w0)], wk_v.at[:, pl.ds(0, w0)])] + [
        cp(SEM_W, x_hbm.at[pl.ds(0, XCH[0]), :], x_v.at[pl.ds(0, XCH[0]), :])]
    cp_xc[0] = [cp(0, wqkv_hbm.at[:, pl.ds(D + w0, D - w0)], wk_v.at[:, pl.ds(w0, D - w0)])]
    last = len(XCH) - 1
    cp_xc[last] += [cp(last, fwd_hbm, fwd_ref), cp(last, shk_hbm, shk_ref),
                    cp(last, dvec_hbm, dvec_ref)]
    cp_epi = [cp(SEM_E, wo_hbm, wo_v), cp(SEM_E, inv_hbm, inv_ref), cp(SEM_E, gw_hbm, gw_ref)]

    def cp_conv(lt):
        static = isinstance(lt, int)
        l0 = lt * 128 if static else pl.multiple_of(lt * 128, 128)
        out = [cp(SEM_C + lt, ssmk_hbm.at[pl.ds(l0, 128), :], ssmk_v.at[lt]),
               cp(SEM_C + lt, bk_hbm.at[:, pl.ds(l0, 128)], bk_v.at[lt]),
               cp(SEM_C + lt, bv_hbm.at[:, pl.ds(l0, 128)], bv_v.at[lt])]
        for i in range(2):
            c = 2 * lt + i
            if static:
                c0 = c * 128 + (D if c >= NL else 0)
            else:
                c0 = pl.multiple_of(c * 128 + jnp.where(c >= NL, D, 0), 128)
            out.append(cp(SEM_C + lt, wqkv_hbm.at[:, pl.ds(c0, 128)], wc_v.at[c]))
        return out

    for grp in [cp_w0] + cp_xc:
        for c_ in grp:
            c_.start()
    for lt in range(NL):
        for c_ in cp_conv(lt):
            c_.start()
    for c_ in cp_epi:
        c_.start()

    zero_s[0:8] = jnp.zeros((8, 128), F32)
    flag_s[...] = jnp.zeros((8, TQ), F32)
    run_s[0] = jnp.int32(1)

    def k_rows(r0, n, l0=0, l1=NL):
        xb = x_v[r0:r0 + n, :]
        if l0 == 0:
            xp_s[r0 // 2:(r0 + n) // 2, :] = pltpu.bitcast(xb, jnp.uint32)
        q4 = n // 4
        s2 = jnp.concatenate(
            [jnp.dot(xb[i * q4:(i + 1) * q4, K4:D], wk_v[K4:D, l0 * 128:l1 * 128],
                     preferred_element_type=F32) for i in range(4)], axis=0)
        return jnp.concatenate(
            [s2[:, (l - l0) * 128:(l - l0 + 1) * 128]
             + jnp.dot(xb[:, 0:K4], wk_v[0:K4, l * 128:(l + 1) * 128], preferred_element_type=F32)
             for l in range(l0, l1)], axis=1)

    def k_store(t, kk):
        r0 = t * TK
        kk = pltpu.bitcast(_to_stored(kk, t).astype(BF16), jnp.uint32)
        for j in range(NP):
            if 40 * j + 48 <= D:
                kj = kk[:, 40 * j:40 * j + 48]
            else:
                kj = jnp.concatenate([kk[:, 40 * j:D], jnp.zeros((TK // 2, 8), jnp.uint32)], axis=1)
            k_s[j, r0 // 2:(r0 + TK) // 2, :] = kj
            v0, v1 = VOF[TC * t] * 8, VOF[TC * t + TC] * 8
            kf = pltpu.bitcast(kj[0:(v1 - v0) // 2], BF16).astype(F32)
            kf_s[j, v0:v1, :] = kf
            if j == 0:
                kfc_s[0, v0:v1, :] = kf
                kr_s[v0:v1, :] = kf

    for c_ in cp_w0:
        c_.wait()
    first = k_rows(0, XCH[0], 0, WK0)
    pend = []
    done = 0
    r0 = 0
    for ci, n in enumerate(XCH):
        for c_ in cp_xc[ci]:
            c_.wait()
        if ci == len(XCH) - 1:
            shk = shk_ref[...].astype(F32)
            dvec = dvec_ref[...].astype(F32).reshape(1, D)
            for lt in range(NL):
                cw_s[lt, 0:4] = shk[:, lt * 128:(lt + 1) * 128]
                cw_s[lt, 8:9] = dvec[:, lt * 128:(lt + 1) * 128]
        end = r0 + n
        while True:
            while (done + 1) * TK <= r0 and (r0 < end or r0 == S):
                allk = jnp.concatenate(pend, axis=0)
                k_store(done, allk[0:TK])
                pend = [allk[TK:]] if allk.shape[0] > TK else []
                done += 1
            if r0 == end:
                break
            m = min(KSUB if r0 < S - KLAST else 128, end - r0, TP - r0 % TP)
            if r0 == 0:
                assert m == XCH[0]
                pend.append(jnp.concatenate([first, k_rows(0, m, WK0, NL)], axis=1))
            else:
                pend.append(k_rows(r0, m))
            r0 += m

    kb_b = (kb0_s, kb1_s)
    G2 = CB // 16
    ROWS = 2 * D // NL

    def make_kb(e, d, z):
        kf = kfc_s[0, 0:NG * 8]
        kb = jnp.broadcast_to(kf[:, DH * e + d:DH * e + d + 1], (NG * 8, 128))
        kb_b[e][pl.ds(z, NG), d] = kb.reshape(NG, 8, 128)

    def conv16(uf, hf, init, gate, sign):
        HB = NB // 2
        acc = [None if init is None else init(a) for a in range(NB)]

        def mac(a, u, h):
            t = u * h
            acc[a] = t if acc[a] is None else (acc[a] + t if sign > 0 else acc[a] - t)

        def block(terms, hs, jg):
            hs = dict(hs)
            hs[jg] = gate(hs[jg])
            for a, tl in terms.items():
                for u, j in [x for x in tl if x[1] != jg] + [x for x in tl if x[1] == jg]:
                    mac(a, u, hs[j])

        hl = {j: hf(j) for j in range(HB)}
        uh = {i: uf(i) for i in range(HB, NB)}
        block({a: [(uh[a - j], j) for j in range(a - HB + 1)] for a in range(HB, NB)}, hl, 0)
        ul = {i: uf(i) for i in range(HB)}
        block({a: [(ul[a - j], j) for j in range(a + 1)] for a in range(HB)}, hl, 0)
        block({a: [(ul[a - j], j) for j in range(HB - 1, a - HB, -1)] for a in range(HB, NB - 1)},
              {j: hl[j] for j in range(1, HB)}, HB - 1)
        hh = {j: hf(j) for j in range(HB, NB)}
        block({a: [(ul[a - j], j) for j in range(HB, a + 1)] for a in range(HB, NB)}, hh, HB)
        return acc

    def chan_body(lt, c):
        for c_ in cp_conv(lt):
            c_.wait()
        z = jnp.minimum(lt, 0)
        fwd = fwd_ref[0]
        cw = cw_s[lt, 0:4]
        st = {"prev": None, "tail": jnp.zeros((8, 128), F32)}
        fwd32 = fwd_ref[1].astype(F32)

        def h_round(a0):
            rhs = jnp.concatenate(
                [ssmk_v[lt, :, (a0 + i) * CB:(a0 + i + 1) * CB] for i in range(4)], axis=0)
            h4 = lax.dot_general(fwd, rhs, _NT, preferred_element_type=F32)
            for i in range(4):
                hh = h4[:, i * 128:(i + 1) * 128].reshape(2 * G2, 2, 8, 128)
                re, im = hh[:, 0], hh[:, 1]
                if st["prev"] is None:
                    re = re + cw_s[lt, 8:9]
                    ore, oim = re, im
                else:
                    pre, pim = st["prev"]
                    ore = jnp.concatenate([re[0:G2] - pim[0:G2], re[G2:] + pim[G2:]], axis=0)
                    oim = jnp.concatenate([im[0:G2] + pre[0:G2], im[G2:] - pre[G2:]], axis=0)
                st["prev"] = (re, im)
                h_s[z, :, 0, a0 + i] = ore
                h_s[z, :, 1, a0 + i] = oim - ore
                h_s[z, :, 2, a0 + i] = oim + ore

        def u_round(a0):
            r0, n = a0 * CB, 4 * CB
            kf = bk_v[lt, r0:r0 + n, :].astype(F32)
            ke = jnp.concatenate([st["tail"], kf], axis=0)
            st["tail"] = kf[n - 8:n]
            k2 = pltpu.roll(ke, 2, 0)
            pe = ke * cw[1:2] + k2 * cw[3:4]
            ks = kf * cw[0:1] + k2[8:] * cw[2:3] + pltpu.roll(pe, 1, 0)[8:]
            kv = ks * bv_v[lt, r0:r0 + n, :].astype(F32)
            rhs = jnp.concatenate([kv[i * CB:(i + 1) * CB] for i in range(4)], axis=1)
            u4 = jnp.dot(fwd32, rhs, preferred_element_type=F32)
            for i in range(4):
                u_s[z, :, :, a0 + i] = u4[:, i * 128:(i + 1) * 128].reshape(2 * G2, 2, 8, 128)

        hc = uc = 0
        for ch in FORDER:
            if ch == "h":
                h_round(4 * hc)
                hc += 1
            else:
                u_round(4 * uc)
                uc += 1
        kr = kr_s[0:NG * 8]
        for dd in range(DH // NL):
            kb0_s[:, lt * (DH // NL) + dd] = jnp.broadcast_to(
                kr[:, dd:dd + 1], (NG * 8, 128)).reshape(NG, 8, 128)
        kr_s[0:NG * 8] = jnp.concatenate([kr[:, DH // NL:], kr[:, 0:DH // NL]], axis=1)
        tiles = []
        for i in range(2):
            wt_s[z, i * 64:(i + 1) * 64, :] = pltpu.bitcast(
                wc_v[2 * lt + i].astype(F32).T.astype(BF16), jnp.uint32)
        ro = pl.multiple_of(lt * ROWS, ROWS)
        for t in range(S // TV):
            s2 = lax.dot_general(
                pltpu.bitcast(wt_s[0, :, K4:D], BF16),
                pltpu.bitcast(xp_s[t * TV // 2:(t + 1) * TV // 2, K4:D], BF16), _NT,
                preferred_element_type=F32)
            for r in range(ROWS // 8):
                tiles.append(s2[r * 8:(r + 1) * 8, 0:128])
            for l in range(TV // 128):
                rl = t * TV + l * 128
                qv = s2[:, l * 128:(l + 1) * 128] + lax.dot_general(
                    pltpu.bitcast(wt_s[0, :, 0:K4], BF16),
                    pltpu.bitcast(xp_s[rl // 2:rl // 2 + 64, 0:K4], BF16), _NT,
                    preferred_element_type=F32)
                for r in range(ROWS // 8):
                    tiles.append(qv[r * 8:(r + 1) * 8])
                qvt_s[pl.ds(ro, ROWS), rl:rl + 128] = qv
        always = zero_s[0:8] == 0.0
        cnt = [0]
        ngate = 12 * 2 * G2

        def gate(v):
            idx = ((cnt[0] - DEP_LEAD) * len(tiles)) // ngate
            cnt[0] += 1
            return v if idx < 0 else jnp.where(always, v, tiles[idx])

        for f in range(2 * G2):
            k1 = conv16(lambda a: u_s[0, f, 0, a] + u_s[0, f, 1, a], lambda a: h_s[0, f, 0, a],
                        None, gate, 1)
            for a in range(NB):
                y_s[lt, a, f, 0] = k1[a]
            yi = conv16(lambda a: u_s[0, f, 0, a], lambda a: h_s[0, f, 1, a],
                        lambda a: y_s[lt, a, f, 0], gate, 1)
            for a in range(NB):
                y_s[lt, a, f, 1] = yi[a]
            yr = conv16(lambda a: u_s[0, f, 1, a], lambda a: h_s[0, f, 2, a],
                        lambda a: y_s[lt, a, f, 0], gate, -1)
            for a in range(NB):
                y_s[lt, a, f, 0] = yr[a]
        return c

    lax.fori_loop(0, NL, chan_body, 0)

    row8 = lax.broadcasted_iota(jnp.int32, (8, TQ), 0)
    row8k = lax.broadcasted_iota(jnp.int32, (8, CK), 0)
    row8s = lax.broadcasted_iota(jnp.int32, (8, S), 0)

    def win(e):
        return 16 * e

    def head_weights(qw, e):
        zeros8 = jnp.zeros((8, qw.shape[1]), F32)
        rows = lax.broadcasted_iota(jnp.int32, (8, qw.shape[1]), 0)
        qw = qw * QSCALE
        if e == 0:
            w = jnp.concatenate([qw[0:16], jnp.where(rows < 4, qw[16:24], 0.0), zeros8], axis=0)
        else:
            w = jnp.concatenate([zeros8, zeros8, jnp.where(rows >= 4, qw[0:8], 0.0),
                                 qw[8:24], zeros8], axis=0)
        return w.astype(BF16)

    def v_window(b, e, k0, n, rows):
        vw = qvt_s[pl.ds(D + b + win(e), 24), k0:k0 + n]
        if e == 0:
            return jnp.concatenate([vw[0:16], jnp.where(rows < 4, vw[16:24], 1.0)], axis=0)
        return jnp.concatenate([jnp.where(rows >= 4, vw[0:8], 1.0), vw[8:24]], axis=0)

    qc_b = (qc0_s, qc1_s)

    def make_q(bx, e, l, z, gate):
        qw = qvt_s[pl.ds(bx + win(e), 24), l * 128:(l + 1) * 128]
        if gate is not None:
            qw = jnp.where(jnp.concatenate([gate[0]] * 3, axis=0), qw,
                           jnp.concatenate([gate[1]] * 3, axis=0))
        qw = (qw * QSCALE).astype(BF16).astype(F32)
        for r_ in range(QREP):
            qc_b[e][r_ + z, :, l * 128:(l + 1) * 128] = qw

    for l in range(S // 128):
        make_q(0, 0, l, 0, None)

    def pv_step(p, acc, restart, bv_, ho_, e, t, cc):
        o = jnp.dot(v_window(bv_, e, cc * CK, CK, row8k), p, preferred_element_type=F32)
        acc = acc + o if restart is None else jnp.where(restart, o, acc)
        if cc == NC - 1:
            ow_s[ho_, :, t * TQ:(t + 1) * TQ] = acc
        return acc

    def attn_fast(j, carry):
        p_prev, acc_prev = carry
        b = pl.multiple_of(40 * j, 8)
        jn = jnp.minimum(j + 1, NP - 1)
        bn = pl.multiple_of(40 * jn, 8)
        z = jnp.minimum(j, 0)
        always = zero_s[0:8] == 0.0
        always_q = jnp.concatenate([always] * (TQ // 128), axis=1)
        items = [(e, t, cc) for e in range(2) for t in range(NT) for cc in range(NC)]
        half = len(items) // 2
        ws = {}
        ps = {}
        pvs = {}
        state = {"acc": None, "rep": 0}

        def qk(n):
            e, t, cc = items[n]
            if cc == 0:
                ws[(t, e)] = head_weights(qvt_s[pl.ds(b + win(e), 24), t * TQ:(t + 1) * TQ], e)
            w = ws[(t, e)]
            kp = k_s[j, MO[cc] * 4:(MO[cc] + MD[cc]) * 4, 0:w.shape[0]]
            s = jnp.dot(pltpu.bitcast(kp, BF16), w, preferred_element_type=F32)
            ps[n] = jnp.exp2(s)

        def vpu(n):
            e, t, cc = items[n]
            for v in range(VOF[cc], VOF[cc + 1]):
                rep = state["rep"] % QREP
                state["rep"] += 1

                def terms(d, kd=None, e=e, t=t, v=v, rep=rep):
                    kd = kb_b[e][v, d] if kd is None else kd
                    return [kd * qc_b[e][rep, pl.ds(4 * e + d, 1), pl.ds(t * TQ + lt * 128, 128)]
                            for lt in range(TQ // 128)]

                def step(d, acc):
                    return [x + y for x, y in zip(acc, terms(d))]

                cols = lax.fori_loop(1, VGD, step, terms(0), unroll=True)
                kg = kb_b[e][v, VGD]
                gn, gr = n - cc + GATES[v][0], GATES[v][1]
                if gn >= 0:
                    dep = ps[gn][gr * 8:gr * 8 + 8, 0:128]
                else:
                    g = [k for k, sv in SRC_OF[NC - 1].items() if sv == ("m", NC + gn, gr)][0]
                    dep = p_prev[g * 8:g * 8 + 8, 0:128]
                kg = jnp.where(always, kg, dep)
                cols = [x + y for x, y in zip(cols, terms(VGD, kg))]
                cols = lax.fori_loop(VGD + 1, DH, step, cols, unroll=True)
                a = jnp.concatenate(cols, axis=1)
                pvs[(n - cc, v)] = jnp.exp2(a)
            m = n % half
            jx, bx, ex = (j, b, 1) if e == 0 else (jn, bn, 0)
            if m % 3 == 2 and m // 3 < DH:
                kfc_s[1 + z, 0:8, :] = ps[n - 1][8:16, 256:256 + 48]
                make_kb(ex, m // 3, z)
            if m == 0 and e == 1:
                kfc_s[0, 0:NG * 8] = kf_s[jx, 0:NG * 8]
            if m % 4 == 1:
                make_q(bx, ex, m // 4, z, (always, ps[n - 1][16:24, 128:256]))

        def p_tile(n):
            cc = items[n][2]
            parts = []
            for g in range(16):
                sv = SRC_OF[cc][g]
                if sv[0] == "v":
                    parts.append(pvs[(n - cc, sv[1])])
                else:
                    parts.append(ps[n - cc + sv[1]][sv[2] * 8:sv[2] * 8 + 8])
            return jnp.concatenate(parts, axis=0)

        for n in range(len(items)):
            qk(n)
            vpu(n)
            if n >= 1:
                e, t, cc = items[n - 1]
                restart = jnp.concatenate([always_q] * 3, axis=0) if cc == 0 else None
                state["acc"] = pv_step(p_tile(n - 1), state["acc"], restart, b, 2 * j + e, e, t, cc)
            else:
                bv_ = pl.multiple_of(40 * jnp.maximum(j - 1, 0), 8)
                ho_ = jnp.where(j == 0, H, 2 * j - 1)
                state["acc"] = pv_step(p_prev, acc_prev, None, bv_, ho_, *items[-1])
        return p_tile(len(items) - 1), state["acc"]

    p_last, acc_last = lax.fori_loop(
        0, NP, attn_fast, (jnp.zeros((CK, TQ), F32), jnp.zeros((24, TQ), F32)), unroll=2)
    pv_step(p_last, acc_last, None, 40 * (NP - 1), H - 1, 1, NT - 1, NC - 1)

    def attn_safe(it, c):
        j = it // (S // TS)
        b = pl.multiple_of(40 * j, 8)
        qs = pl.ds(pl.multiple_of((it % (S // TS)) * TS, TS), TS)
        for e in range(2):
            w = head_weights(qvt_s[pl.ds(b + win(e), 24), qs], e)
            s = jnp.dot(pltpu.bitcast(k_s[j, :, 0:w.shape[0]], BF16), w,
                        preferred_element_type=F32)
            m = jnp.max(s, axis=0, keepdims=True)
            p = _to_natural(jnp.exp2(s - m))
            ow_s[2 * j + e, :, qs] = jnp.dot(v_window(b, e, 0, S, row8s), p,
                                             preferred_element_type=F32)
        return c

    for c_ in cp_epi:
        c_.wait()

    def epi_body(t, c):
        r0 = pl.multiple_of(t * TP, TP)
        always = zero_s[0:8] == 0.0

        def gated(v, tile):
            n = v.shape[1] // 128
            return jnp.where(jnp.concatenate([always] * n, axis=1), v,
                             jnp.concatenate([tile] * n, axis=1))

        inv = inv_ref[...].astype(F32)
        HC = CB // 2
        sub = lax.broadcasted_iota(jnp.int32, (8, 256), 0)

        def rev8(v):
            v = pltpu.roll(v, 4, 0)
            v = jnp.where((sub & 2) == 0, pltpu.roll(v, 6, 0), pltpu.roll(v, 2, 0))
            return jnp.where((sub & 1) == 0, pltpu.roll(v, 7, 0), pltpu.roll(v, 1, 0))

        ycols = [[None] * NL for _ in range(TP // CB)]
        ytiles = []
        for i in range(0, TP // CB, 2):
            for lt in range(NL):
                cs = [jnp.dot(inv[ri * HC:(ri + 1) * HC],
                              jnp.concatenate(
                                  [y_s[lt, t * (TP // CB) + i + k, :, ri].reshape(CB, 128)
                                   for k in range(2)], axis=1),
                              preferred_element_type=F32) for ri in range(2)]
                up = cs[0] - cs[1]
                lo = cs[0] + cs[1]
                ytiles += [up[r * 8:(r + 1) * 8, 0:128] for r in range(0, HC // 8, 2)]
                lo = jnp.concatenate([rev8(lo[r * 8:(r + 1) * 8])
                                      for r in reversed(range(HC // 8))], axis=0)
                yy = jnp.concatenate([lo, up], axis=0)
                for k in range(2):
                    ycols[i + k][lt] = yy[:, k * 128:(k + 1) * 128]
        ys = [jnp.concatenate(ycols[i], axis=1) for i in range(TP // CB)]
        rows = [None] * NP
        for n, j in enumerate([12, 13, 14, 15] + list(range(12))):
            oe = ow_s[2 * j, :, pl.ds(r0, TP)]
            oo = ow_s[2 * j + 1, :, pl.ds(r0, TP)]
            den = jnp.where(row8 < 4, oo[0:8], oe[16:24])
            gi = ((n - EG_LEAD) * len(ytiles)) // EG_SPAN
            if gi >= 0:
                den = gated(den, ytiles[gi])
            rec = pl.reciprocal(den, approx=True)
            rec = rec * (2.0 - den * rec)
            mid = jnp.where(row8 < 4, oe[16:24], oo[0:8])
            re_, ro_ = rec[4:5], rec[0:1]
            rows[j] = jnp.concatenate(
                [oe[0:16] * re_, mid * pltpu.roll(rec, 4, 0), oo[8:24] * ro_], axis=0)
        o = jnp.concatenate(rows, axis=0).astype(BF16).T
        q4 = TP // 4
        s2 = jnp.concatenate(
            [jnp.dot(o[i * q4:(i + 1) * q4, K4:D], wo_v[K4:D, :], preferred_element_type=F32)
             for i in range(4)], axis=0)
        gw8 = jnp.broadcast_to(gw_ref[...].astype(F32).reshape(1, D), (8, D))
        gs = []
        for i in range(TP // CB):
            rr = pl.multiple_of(r0 + i * CB, CB)
            gwi = gated(gw8, ytiles[len(ytiles) - 1 - (3 - i) * EG_X])[0:1]
            z = jnp.sum(x_v[pl.ds(rr, CB), :].astype(F32) * gwi, axis=-1, keepdims=True)
            gs.append(1.0 / (1.0 + jnp.exp(-z)))
        g = jnp.concatenate(gs, axis=0)
        y = jnp.concatenate(ys, axis=0)
        bad = flag_s[...]
        for l in range(NL):
            ls = slice(l * 128, (l + 1) * 128)
            a = s2[:, ls] + jnp.dot(o[:, 0:K4], wo_v[0:K4, ls], preferred_element_type=F32)
            b = x_v[pl.ds(r0, TP), ls].astype(F32) * y[:, ls]
            o_v[pl.ds(r0, TP), ls] = (g * a + (1.0 - g) * b).astype(BF16)
            cp(0, o_v.at[pl.ds(r0, TP), pl.ds(l * 128, 128)],
               o_hbm.at[pl.ds(r0, TP), pl.ds(l * 128, 128)]).start()
            for k in range(8):
                h = 8 * l + k
                if h >= H:
                    break
                hi = gated(jnp.full((8, TP), SAFE_HI, F32), a[k * 64:k * 64 + 8])
                w = ow_s[h, :, pl.ds(r0, TP)]
                ok = (jnp.abs(w[0:8]) <= hi) & (jnp.abs(w[8:16]) <= hi) & (jnp.abs(w[16:24]) <= hi)
                if h % 2 == 0:
                    ok = ok & ((row8 < 4) | (w[16:24] >= SAFE_LO))
                else:
                    ok = ok & ((row8 >= 4) | (w[0:8] >= SAFE_LO))
                bad = jnp.where(ok, bad, 1.0)
        flag_s[...] = bad
        return c

    def attempt(i, c):
        @pl.when(run_s[0] > 0)
        def _():
            @pl.when(i == 1)
            def _():
                lax.fori_loop(0, NP * (S // TS), attn_safe, 0)

            lax.fori_loop(0, NX, epi_body, 0)
            run_s[0] = (jnp.max(flag_s[...]) > 0.0).astype(jnp.int32)
            cp(0, o_v, o_hbm).wait()

        return c

    lax.fori_loop(0, 2, attempt, 0)


@jax.jit
def pallas_gated_mix__mha_block__ssm_conv_h3__prompt_kernel(
    A_x: jax.Array,
    A_wqkv: jax.Array,
    A_wo: jax.Array,
    B_q: jax.Array,
    B_k: jax.Array,
    B_v: jax.Array,
    B_shift_k: jax.Array,
    B_ssm_k: jax.Array,
    B_ssm_D: jax.Array,
    gate_w: jax.Array,
):
    del B_q
    fwd, inv = _dft_mats()
    hbm = pl.BlockSpec(memory_space=pl.ANY)
    out = pl.pallas_call(
        _kernel,
        out_shape=jax.ShapeDtypeStruct((S, D), BF16),
        in_specs=[hbm] * 11,
        out_specs=hbm,
        scratch_shapes=[
            pltpu.VMEM((S, D), BF16),
            pltpu.VMEM((D, D), BF16),
            pltpu.VMEM((2 * NL, D, 128), BF16),
            pltpu.VMEM((D, D), BF16),
            pltpu.VMEM((NL, S, 128), BF16),
            pltpu.VMEM((NL, S, 128), BF16),
            pltpu.VMEM((NL, 128, S), BF16),
            pltpu.VMEM((S, D), BF16),
            pltpu.SemaphoreType.DMA((len(XCH) + 2 + NL,)),
            pltpu.VMEM((1, 128, D), jnp.uint32),
            pltpu.VMEM((S // 2, D), jnp.uint32),
            pltpu.VMEM((NP, S // 2, 48), jnp.uint32),
            pltpu.VMEM((2 * D, S), F32),
            pltpu.VMEM((H + 1, 24, S), F32),
            pltpu.VMEM((1, CB // 8, 2, NB, 8, 128), F32),
            pltpu.VMEM((1, CB // 8, 3, NB, 8, 128), F32),
            pltpu.VMEM((NL, NB, CB // 8, 2, 8, 128), F32),
            pltpu.VMEM((NL, 32, 128), F32),
            pltpu.VMEM((8, TQ), F32),
            pltpu.VMEM((32, 128), F32),
            pltpu.VMEM((NG, DH, 8, 128), F32),
            pltpu.VMEM((NG, DH, 8, 128), F32),
            pltpu.VMEM((QREP, 24, S), F32),
            pltpu.VMEM((QREP, 24, S), F32),
            pltpu.VMEM((NP, NGP * 8, 48), F32),
            pltpu.VMEM((2, NGP * 8, 48), F32),
            pltpu.VMEM((NGP * 8, 48), F32),
            pltpu.VMEM((2, 2 * CB, CB), BF16),
            pltpu.VMEM((CB, CB), BF16),
            pltpu.VMEM((4, D), BF16),
            pltpu.VMEM((D,), BF16),
            pltpu.VMEM((D,), BF16),
            pltpu.SMEM((1,), jnp.int32),
        ],
        compiler_params=pltpu.CompilerParams(vmem_limit_bytes=120 * 1024 * 1024),
    )(
        A_x.reshape(S, D), A_wqkv, A_wo, B_k.reshape(S, D), B_v.reshape(S, D), B_ssm_k,
        B_shift_k.T, B_ssm_D, gate_w, fwd, inv,
    )
    return out.reshape(1, S, D)
```
